```python
import os as _os
_os.environ.setdefault("JAX_PLATFORMS", "cpu")
import jax
import jax.numpy as jnp

def _softmax(x, axis=-1):
    return jax.nn.softmax(x, axis=axis)
def _gelu(x):
    return jax.nn.gelu(x, approximate=True)
def _silu(x):
    return jax.nn.silu(x)
def _sigmoid(x):
    return jax.nn.sigmoid(x)
def _layernorm(x, axis=-1, eps=1e-5):
    m = jnp.mean(x, axis=axis, keepdims=True)
    v = jnp.var(x, axis=axis, keepdims=True)
    return (x - m) / jnp.sqrt(v + eps)
def _scatter_add(tgt, idx, src, axis=0):
    return tgt.at[idx].add(src)
def _segment_sum(src, seg, n):
    return jax.ops.segment_sum(src, seg, n)
class _Rng:
    def __init__(self, key):
        self._k = key
    def _next(self):
        self._k, sub = jax.random.split(self._k)
        return sub
    def normal(self, shape):
        return jax.random.normal(self._next(), shape, dtype=jnp.bfloat16)
    def randint(self, lo, hi, shape):
        return jax.random.randint(self._next(), shape, lo, hi, dtype=jnp.int32)
    def uniform(self, shape, lo=0.0, hi=1.0):
        return jax.random.uniform(self._next(), shape, jnp.bfloat16, lo, hi)
    def permutation(self, n):
        return jax.random.permutation(self._next(), n)


kernel_name = 'standalone__linear_kernel_hedgehog__prompt'

def setup_inputs():
    _rng = _Rng(jax.random.key(int.from_bytes(__import__("os").urandom(4), "little")))
    _w = (lambda a: (lambda t: t.astype(jnp.bfloat16) if jnp.issubdtype(t.dtype, jnp.floating) else t)(jnp.asarray(a)))
    B, S, D, H = 1, 2048, 1024, 32
    Dh = D // H
    return {
        "x": _w((lambda *s: _rng.normal(s) * 0.4)(B, S, D)),
        "wqkv": _w((lambda *s: _rng.normal(s) * 0.4)(D, 3 * D)),
        "w_phi": _w((lambda *s: _rng.normal(s) * 0.4)(H, Dh, Dh) * (Dh ** -0.5)),
        "wo": _w((lambda *s: _rng.normal(s) * 0.05)(D, D)),
    }

def reference(x, wqkv, w_phi, wo):
    B, S, D = x.shape
    H = 32; Dh = D // H
    qkv = (lambda x, *d: x.transpose(*d))((x @ wqkv).reshape(B, S, 3, H, Dh), 2, 0, 3, 1, 4)
    q, k, v = qkv[0], qkv[1], qkv[2]
    pq = jnp.einsum("bhsd,hdf->bhsf", q, w_phi)
    pk = jnp.einsum("bhsd,hdf->bhsf", k, w_phi)
    phi_q = jnp.concatenate([_softmax(pq, axis=-1), _softmax(-pq, axis=-1)], axis=-1)
    phi_k = jnp.concatenate([_softmax(pk, axis=-1), _softmax(-pk, axis=-1)], axis=-1)
    kv = jnp.einsum("bhsf,bhsd->bhfd", phi_k, v)
    z  = jnp.einsum("bhsf->bhf", phi_k)
    num = jnp.einsum("bhqf,bhfd->bhqd", phi_q, kv)
    den = jnp.einsum("bhqf,bhf->bhq", phi_q, z)[..., None] + 1e-6
    o = num / den
    return (lambda x, *d: x.transpose(*d))(o, 0, 2, 1, 3).reshape(B, S, D) @ wo
```

```python
import functools
import jax
import jax.numpy as jnp
from jax import lax
import jax.experimental.pallas as pl
import jax.experimental.pallas.tpu as pltpu

H = 32
DH = 32
G = 128
HPG = G // DH

_NT = (((1,), (1,)), ((), ()))
_NN = (((1,), (0,)), ((), ()))


def _dual_softmax_t(p):
    rows, t = p.shape
    p3 = p.reshape(rows // DH, DH, t)
    mx = jnp.max(p3, axis=1, keepdims=True)
    mn = jnp.min(p3, axis=1, keepdims=True)
    ep = jnp.exp(p3 - mx)
    en = jnp.exp(mn - p3)
    sp = jnp.sum(ep, axis=1, keepdims=True)
    sn = jnp.sum(en, axis=1, keepdims=True)
    fp = (ep * (1.0 / sp)).reshape(rows, t)
    fn = (en * (1.0 / sn)).reshape(rows, t)
    return fp, fn


def _kernel(x_ref, wq_ref, wk_ref, wv_ref, wphi_ref, wo_ref, o_ref,
            wkt_s, wqt_s, kv_s, z_s, lhs_s, *, n_s, ts, d):
    j = pl.program_id(0)
    ng = d // G

    def fold(w_ref, out_s):
        r = lax.broadcasted_iota(jnp.int32, (G, G), 0)
        c = lax.broadcasted_iota(jnp.int32, (G, G), 1)
        same_head = (r // DH) == (c // DH)
        fr = lax.broadcasted_iota(jnp.int32, (DH, G), 0)
        fc = lax.broadcasted_iota(jnp.int32, (DH, G), 1)
        expand = jnp.where(fr == (fc % DH), 1.0, 0.0).astype(jnp.bfloat16)
        for g in range(ng):
            wrows = wphi_ref[g * G:(g + 1) * G, :]
            tiled = lax.dot_general(wrows, expand, _NN,
                                    preferred_element_type=jnp.float32)
            bd = jnp.where(same_head, tiled, 0.0)
            bdt = bd.T.astype(jnp.bfloat16)
            wcols = w_ref[:, g * G:(g + 1) * G]
            out_s[g * G:(g + 1) * G, :] = lax.dot_general(
                bdt, wcols, _NT, preferred_element_type=jnp.float32).astype(out_s.dtype)

    @pl.when(j == 0)
    def _():
        fold(wk_ref, wkt_s)
        fold(wq_ref, wqt_s)
        kv_s[...] = jnp.zeros(kv_s.shape, kv_s.dtype)
        z_s[...] = jnp.zeros(z_s.shape, z_s.dtype)

    @pl.when(j < n_s)
    def _():
        x = x_ref[...]
        pk = lax.dot_general(wkt_s[...], x, _NT, preferred_element_type=jnp.float32)
        v = lax.dot_general(x, wv_ref[...], _NN,
                            preferred_element_type=jnp.float32).astype(jnp.bfloat16)
        fp, fn = _dual_softmax_t(pk)
        zp = fp[:, 0:G]
        zn = fn[:, 0:G]
        for c in range(1, ts // G):
            zp = zp + fp[:, c * G:(c + 1) * G]
            zn = zn + fn[:, c * G:(c + 1) * G]
        z_s[0:d, :] += zp
        z_s[d:2 * d, :] += zn
        fpb = fp.astype(jnp.bfloat16)
        fnb = fn.astype(jnp.bfloat16)
        for g in range(ng):
            lhs = jnp.concatenate([fpb[g * G:(g + 1) * G], fnb[g * G:(g + 1) * G]], axis=0)
            kv_s[g] += lax.dot_general(lhs, v[:, g * G:(g + 1) * G], _NN,
                                       preferred_element_type=jnp.float32)

    @pl.when(j == n_s)
    def _():
        r = lax.broadcasted_iota(jnp.int32, (2 * G, G), 0)
        c = lax.broadcasted_iota(jnp.int32, (2 * G, G), 1)
        fhead = (r % G) // DH
        for g in range(ng):
            kv = jnp.where(fhead == (c // DH), kv_s[g], 0.0)
            zg = jnp.concatenate([z_s[g * G:(g + 1) * G, :], z_s[d + g * G:d + (g + 1) * G, :]],
                                 axis=0)
            zsum = jnp.sum(zg, axis=1, keepdims=True)
            zcol = jnp.where(fhead == c, jnp.broadcast_to(zsum, (2 * G, G)), 0.0)
            both = jnp.concatenate([kv, zcol], axis=1)
            lhs_s[g] = both.T.astype(jnp.bfloat16)

    @pl.when(j >= n_s)
    def _():
        x = x_ref[...]
        pq = lax.dot_general(wqt_s[...], x, _NT, preferred_element_type=jnp.float32)
        fp, fn = _dual_softmax_t(pq)
        fpb = fp.astype(jnp.bfloat16)
        fnb = fn.astype(jnp.bfloat16)
        outs = []
        for g in range(ng):
            rhs = jnp.concatenate([fpb[g * G:(g + 1) * G], fnb[g * G:(g + 1) * G]], axis=0)
            r = lax.dot_general(lhs_s[g, 0:G + 16, :], rhs, _NN,
                                preferred_element_type=jnp.float32)
            num = r[0:G].reshape(HPG, DH, ts)
            den = r[G:G + HPG].reshape(HPG, 1, ts) + 1e-6
            outs.append((num / den).reshape(G, ts))
        ot = jnp.concatenate(outs, axis=0)
        o = ot.T.astype(jnp.bfloat16)
        o_ref[...] = lax.dot_general(o, wo_ref[...], _NN,
                                     preferred_element_type=jnp.float32).astype(o_ref.dtype)


@jax.jit
def pallas_standalone__linear_kernel_hedgehog__prompt_kernel(x, wqkv, w_phi, wo):
    b, s, d = x.shape
    assert b == 1 and d == H * DH
    ts = 512
    n_s = s // ts
    x2 = x.reshape(s, d)
    wphi2 = w_phi.reshape(d, DH)
    ng = d // G
    kern = functools.partial(_kernel, n_s=n_s, ts=ts, d=d)
    out = pl.pallas_call(
        kern,
        grid=(2 * n_s,),
        in_specs=[
            pl.BlockSpec((ts, d), lambda j: (j % n_s, 0)),
            pl.BlockSpec((d, d), lambda j: (0, 0)),
            pl.BlockSpec((d, d), lambda j: (0, 1)),
            pl.BlockSpec((d, d), lambda j: (0, 2)),
            pl.BlockSpec((d, DH), lambda j: (0, 0)),
            pl.BlockSpec((d, d), lambda j: (0, 0)),
        ],
        out_specs=pl.BlockSpec((ts, d), lambda j: (jnp.maximum(j - n_s, 0), 0)),
        out_shape=jax.ShapeDtypeStruct((s, d), x.dtype),
        scratch_shapes=[
            pltpu.VMEM((d, d), jnp.bfloat16),
            pltpu.VMEM((d, d), jnp.bfloat16),
            pltpu.VMEM((ng, 2 * G, G), jnp.float32),
            pltpu.VMEM((2 * d, G), jnp.float32),
            pltpu.VMEM((ng, 2 * G, 2 * G), jnp.bfloat16),
        ],
        compiler_params=pltpu.CompilerParams(
            dimension_semantics=("arbitrary",),
            vmem_limit_bytes=100 * 1024 * 1024,
        ),
    )(x2, wqkv, wqkv, wqkv, wphi2, wo)
    return out.reshape(b, s, d)
```

```python
import functools
import jax
import jax.numpy as jnp
from jax import lax
import jax.experimental.pallas as pl
import jax.experimental.pallas.tpu as pltpu

H = 32
DH = 32
G = 128
PR = 80
WV_CHUNKS = (256, 256, 512)
OC = 256

_NT = (((1,), (1,)), ((), ()))
_NN = (((1,), (0,)), ((), ()))


def _dual_softmax_t(p):
    rows, t = p.shape
    p3 = p.reshape(rows // DH, DH, t)
    mx = jnp.max(p3, axis=1, keepdims=True)
    mn = jnp.min(p3, axis=1, keepdims=True)
    ep = jnp.exp(p3 - mx)
    en = jnp.exp(mn - p3)
    sp = jnp.sum(ep, axis=1, keepdims=True)
    sn = jnp.sum(en, axis=1, keepdims=True)
    fp = (ep * (1.0 / sp)).reshape(rows, t)
    fn = (en * (1.0 / sn)).reshape(rows, t)
    return fp, fn


def _pair_rhs(fpb, fnb, p):
    a = 2 * p * DH
    return jnp.concatenate([fpb[a:a + DH], fnb[a:a + DH],
                            fpb[a + DH:a + 2 * DH], fnb[a + DH:a + 2 * DH]], axis=0)


def _kernel(x_hbm, wqkv_hbm, wphi_hbm, wo_hbm, o_hbm,
            x_s, wphi_s, wq_s, wk_s, wv_s, wo_s, wkt_s, wqt_s, wvt_s, v0_s, kv_s, z_s, lhs_s,
            out_s, sems, xsems, osems, *, n_s, ts, d):
    j = pl.program_id(0)
    ng = d // G
    npair = H // 2
    noc = d // OC
    wv_off = [sum(WV_CHUNKS[:i]) for i in range(len(WV_CHUNKS))]

    def wv_copy(i):
        return pltpu.make_async_copy(
            wqkv_hbm.at[:, pl.ds(2 * d + wv_off[i], WV_CHUNKS[i])],
            wv_s.at[:, pl.ds(wv_off[i], WV_CHUNKS[i])], sems.at[4 + i])

    def wk_copy():
        return pltpu.make_async_copy(wqkv_hbm.at[:, pl.ds(d, d)], wk_s, sems.at[0])

    def wq_copy():
        return pltpu.make_async_copy(wqkv_hbm.at[:, pl.ds(0, d)], wq_s, sems.at[1])

    def wo_copy():
        return pltpu.make_async_copy(wo_hbm, wo_s, sems.at[2])

    def wphi_copy():
        return pltpu.make_async_copy(wphi_hbm, wphi_s, sems.at[3])

    def x_copy(blk):
        start = pl.multiple_of(blk * ts, ts)
        return pltpu.make_async_copy(x_hbm.at[pl.ds(start, ts), :], x_s.at[pl.ds(start, ts), :],
                                     xsems.at[blk])

    def out_copy(blk, c):
        start = pl.multiple_of(blk * ts, ts)
        return pltpu.make_async_copy(out_s.at[pl.ds(start, ts), pl.ds(c * OC, OC)],
                                     o_hbm.at[pl.ds(start, ts), pl.ds(c * OC, OC)],
                                     osems.at[blk * noc + c])

    def load_x(blk):
        return x_s[pl.ds(pl.multiple_of(blk * ts, ts), ts), :]

    def bd_t():
        fr = lax.broadcasted_iota(jnp.int32, (G, DH), 0)
        fc = lax.broadcasted_iota(jnp.int32, (G, DH), 1)
        expand_t = jnp.where((fr % DH) == fc, 1.0, 0.0).astype(jnp.bfloat16)
        tiled = lax.dot_general(expand_t, wphi_s[...], _NT,
                                preferred_element_type=jnp.float32)
        r = lax.broadcasted_iota(jnp.int32, (G, d), 0)
        c = lax.broadcasted_iota(jnp.int32, (G, d), 1)
        same_head = (r // DH) == ((c % G) // DH)
        return jnp.where(same_head, tiled, 0.0).astype(jnp.bfloat16)

    def fold_group(bdt, w_s, out_ref, g):
        out_ref[g * G:(g + 1) * G, :] = lax.dot_general(
            bdt[:, g * G:(g + 1) * G], w_s[:, g * G:(g + 1) * G], _NT,
            preferred_element_type=jnp.float32).astype(out_ref.dtype)

    def xh_copy(h):
        hs = ts // 2
        return pltpu.make_async_copy(x_hbm.at[pl.ds(h * hs, hs), :], x_s.at[pl.ds(h * hs, hs), :],
                                     sems.at[4 + len(WV_CHUNKS) + h])

    @pl.when(j == 0)
    def _():
        hs = ts // 2
        xh_copy(0).start()
        wv_copy(0).start()
        kv_s[...] = jnp.zeros(kv_s.shape, kv_s.dtype)
        z_s[...] = jnp.zeros(z_s.shape, z_s.dtype)
        wv_copy(0).wait()
        xh_copy(0).wait()
        xh_copy(1).start()
        wv_copy(1).start()
        c0 = WV_CHUNKS[0]
        wt0 = wv_s[:, 0:c0].astype(jnp.float32).T.astype(jnp.bfloat16)
        wvt_s[0:c0, :] = wt0
        v0_s[0:c0, 0:hs] = lax.dot_general(
            wt0, x_s[0:hs, :], _NT, preferred_element_type=jnp.float32).astype(jnp.bfloat16)
        xh_copy(1).wait()
        wv_copy(2).start()
        v0_s[0:c0, hs:ts] = lax.dot_general(
            wt0, x_s[hs:ts, :], _NT, preferred_element_type=jnp.float32).astype(jnp.bfloat16)
        x = x_s[0:ts, :]
        for i in range(1, len(WV_CHUNKS)):
            wv_copy(i).wait()
            if i == 1:
                wphi_copy().start()
                wk_copy().start()
            if i == 2:
                for blk in range(1, n_s):
                    x_copy(blk).start()
                wq_copy().start()
                wo_copy().start()
            lo, hi = wv_off[i], wv_off[i] + WV_CHUNKS[i]
            wt = wv_s[:, lo:hi].astype(jnp.float32).T.astype(jnp.bfloat16)
            wvt_s[lo:hi, :] = wt
            v0_s[lo:hi, :] = lax.dot_general(
                wt, x, _NT, preferred_element_type=jnp.float32).astype(jnp.bfloat16)
        wphi_copy().wait()
        wk_copy().wait()
        bdt = bd_t()
        for g in range(ng):
            fold_group(bdt, wk_s, wkt_s, g)

    def phase1(first):
        x = load_x(j - 1)
        pk = lax.dot_general(wkt_s[...], x, _NT, preferred_element_type=jnp.float32)
        if first:
            vt = v0_s[...]
        else:
            vt = lax.dot_general(wvt_s[...], x, _NT,
                                 preferred_element_type=jnp.float32).astype(jnp.bfloat16)
        fp, fn = _dual_softmax_t(pk)
        zp = fp[:, 0:G]
        zn = fn[:, 0:G]
        for c in range(1, ts // G):
            zp = zp + fp[:, c * G:(c + 1) * G]
            zn = zn + fn[:, c * G:(c + 1) * G]
        z_s[0:d, :] += zp
        z_s[d:2 * d, :] += zn
        fpb = fp.astype(jnp.bfloat16)
        fnb = fn.astype(jnp.bfloat16)
        for p in range(npair):
            kv_s[p] += lax.dot_general(vt[2 * p * DH:(2 * p + 2) * DH], _pair_rhs(fpb, fnb, p),
                                       _NT, preferred_element_type=jnp.float32)

    @pl.when(j == 1)
    def _():
        phase1(True)

    @pl.when(jnp.logical_and(j >= 2, j <= n_s))
    def _():
        x_copy(j - 1).wait()
        phase1(False)

    @pl.when(j == n_s + 1)
    def _():
        wq_copy().wait()
        wo_copy().wait()
        bdt = bd_t()
        for g in range(ng):
            fold_group(bdt, wq_s, wqt_s, g)
        r = lax.broadcasted_iota(jnp.int32, (2 * DH, G), 0)
        c = lax.broadcasted_iota(jnp.int32, (2 * DH, G), 1)
        same_head = (r // DH) == (c // (2 * DH))
        rr = lax.broadcasted_iota(jnp.int32, (16, G), 0)
        cc = lax.broadcasted_iota(jnp.int32, (16, G), 1)
        den_mask = rr == (cc // (2 * DH))
        zall_p = z_s[0:d, :]
        zall_n = z_s[d:2 * d, :]
        for p in range(npair):
            kvm = jnp.where(same_head, kv_s[p], 0.0)
            zt = _pair_rhs(zall_p, zall_n, p).T
            zrow = jnp.sum(zt, axis=0, keepdims=True)
            den_rows = jnp.where(den_mask, jnp.broadcast_to(zrow, (16, G)), 0.0)
            lhs_s[p] = jnp.concatenate([kvm, den_rows], axis=0).astype(jnp.bfloat16)

    @pl.when(j >= n_s + 1)
    def _():
        blk = j - 1 - n_s
        x = load_x(blk)
        pq = lax.dot_general(wqt_s[...], x, _NT, preferred_element_type=jnp.float32)
        fp, fn = _dual_softmax_t(pq)
        fpb = fp.astype(jnp.bfloat16)
        fnb = fn.astype(jnp.bfloat16)
        outs = []
        for p in range(npair):
            r = lax.dot_general(lhs_s[p], _pair_rhs(fpb, fnb, p), _NN,
                                preferred_element_type=jnp.float32)
            num = r[0:2 * DH].reshape(2, DH, ts)
            den = r[2 * DH:2 * DH + 2].reshape(2, 1, ts) + 1e-6
            outs.append((num / den).reshape(2 * DH, ts))
        ot = jnp.concatenate(outs, axis=0)
        o = ot.T.astype(jnp.bfloat16)
        start = pl.multiple_of(blk * ts, ts)
        for c in range(noc):
            out_s[pl.ds(start, ts), c * OC:(c + 1) * OC] = lax.dot_general(
                o, wo_s[:, c * OC:(c + 1) * OC], _NN,
                preferred_element_type=jnp.float32).astype(out_s.dtype)
            out_copy(blk, c).start()

    @pl.when(j == 2 * n_s)
    def _():
        for blk in range(n_s):
            for c in range(noc):
                out_copy(blk, c).wait()


@jax.jit
def pallas_standalone__linear_kernel_hedgehog__prompt_kernel(x, wqkv, w_phi, wo):
    b, s, d = x.shape
    assert b == 1 and d == H * DH
    ts = 512
    n_s = s // ts
    x2 = x.reshape(s, d)
    wphi2 = w_phi.reshape(d, DH)
    kern = functools.partial(_kernel, n_s=n_s, ts=ts, d=d)
    out = pl.pallas_call(
        kern,
        grid=(2 * n_s + 1,),
        in_specs=[
            pl.BlockSpec(memory_space=pl.ANY),
            pl.BlockSpec(memory_space=pl.ANY),
            pl.BlockSpec(memory_space=pl.ANY),
            pl.BlockSpec(memory_space=pl.ANY),
        ],
        out_specs=pl.BlockSpec(memory_space=pl.ANY),
        out_shape=jax.ShapeDtypeStruct((s, d), x.dtype),
        scratch_shapes=[
            pltpu.VMEM((s, d), jnp.bfloat16),
            pltpu.VMEM((d, DH), jnp.bfloat16),
            pltpu.VMEM((d, d), jnp.bfloat16),
            pltpu.VMEM((d, d), jnp.bfloat16),
            pltpu.VMEM((d, d), jnp.bfloat16),
            pltpu.VMEM((d, d), jnp.bfloat16),
            pltpu.VMEM((d, d), jnp.bfloat16),
            pltpu.VMEM((d, d), jnp.bfloat16),
            pltpu.VMEM((d, d), jnp.bfloat16),
            pltpu.VMEM((d, ts), jnp.bfloat16),
            pltpu.VMEM((H // 2, 2 * DH, G), jnp.float32),
            pltpu.VMEM((2 * d, G), jnp.float32),
            pltpu.VMEM((H // 2, PR, G), jnp.bfloat16),
            pltpu.VMEM((s, d), jnp.bfloat16),
            pltpu.SemaphoreType.DMA((6 + len(WV_CHUNKS),)),
            pltpu.SemaphoreType.DMA((n_s,)),
            pltpu.SemaphoreType.DMA((n_s * (d // OC),)),
        ],
        compiler_params=pltpu.CompilerParams(
            dimension_semantics=("arbitrary",),
            vmem_limit_bytes=100 * 1024 * 1024,
        ),
    )(x2, wqkv, wphi2, wo)
    return out.reshape(b, s, d)
```

```python
import functools

import jax
import jax.numpy as jnp
from jax import lax
import jax.experimental.pallas as pl
import jax.experimental.pallas.tpu as pltpu

H = 32
DH = 32
G = 128
WV_CHUNKS = (256, 256, 512)
X_CHUNKS = (128, 128, 256)
AHEAD = 2
OC = 256

_NT = (((1,), (1,)), ((), ()))
_NN = (((1,), (0,)), ((), ()))


def _dual_softmax_t(p):
    rows, t = p.shape
    p3 = p.reshape(rows // DH, DH, t)
    mx = jnp.max(p3, axis=1, keepdims=True)
    mn = jnp.min(p3, axis=1, keepdims=True)
    ep = jnp.exp(p3 - mx)
    en = jnp.exp(mn - p3)
    sp = jnp.sum(ep, axis=1, keepdims=True)
    sn = jnp.sum(en, axis=1, keepdims=True)
    fp = (ep * (1.0 / sp)).reshape(rows, t)
    fn = (en * (1.0 / sn)).reshape(rows, t)
    return fp, fn


def _pair_rhs(fpb, fnb, p):
    a = 2 * p * DH
    return jnp.concatenate([fpb[a:a + DH], fnb[a:a + DH],
                            fpb[a + DH:a + 2 * DH], fnb[a + DH:a + 2 * DH]], axis=0)


def _kernel(x_hbm, wqkv_hbm, wphi_hbm, wo_hbm, o_hbm,
            x_s, wphi_s, wq_s, wk_s, wv_s, wo_s, wkt_s, wqt_s, wvt_s, v0_s, kv_s, z_s, lhs_s,
            out_s, sems, xsems, osems, *, n_s, ts, d):
    j = pl.program_id(0)
    ng = d // G
    npair = H // 2
    noc = d // OC
    wv_off = [sum(WV_CHUNKS[:i]) for i in range(len(WV_CHUNKS))]

    def wv_copy(i):
        return pltpu.make_async_copy(
            wqkv_hbm.at[:, pl.ds(2 * d + wv_off[i], WV_CHUNKS[i])],
            wv_s.at[:, pl.ds(wv_off[i], WV_CHUNKS[i])], sems.at[4 + i])

    def wk_copy():
        return pltpu.make_async_copy(wqkv_hbm.at[:, pl.ds(d, d)], wk_s, sems.at[0])

    def wq_copy():
        return pltpu.make_async_copy(wqkv_hbm.at[:, pl.ds(0, d)], wq_s, sems.at[1])

    def wo_copy():
        return pltpu.make_async_copy(wo_hbm, wo_s, sems.at[2])

    def wphi_copy():
        return pltpu.make_async_copy(wphi_hbm, wphi_s, sems.at[3])

    def x_copy(blk):
        start = pl.multiple_of(blk * ts, ts)
        return pltpu.make_async_copy(x_hbm.at[pl.ds(start, ts), :], x_s.at[pl.ds(start, ts), :],
                                     xsems.at[blk])

    def out_copy(blk, c):
        start = pl.multiple_of(blk * ts, ts)
        return pltpu.make_async_copy(out_s.at[pl.ds(start, ts), pl.ds(c * OC, OC)],
                                     o_hbm.at[pl.ds(start, ts), pl.ds(c * OC, OC)],
                                     osems.at[blk * noc + c])

    def load_x(blk):
        return x_s[pl.ds(pl.multiple_of(blk * ts, ts), ts), :]

    def bd_t():
        fr = lax.broadcasted_iota(jnp.int32, (G, DH), 0)
        fc = lax.broadcasted_iota(jnp.int32, (G, DH), 1)
        expand_t = jnp.where((fr % DH) == fc, 1.0, 0.0).astype(jnp.bfloat16)
        tiled = lax.dot_general(expand_t, wphi_s[...], _NT,
                                preferred_element_type=jnp.float32)
        r = lax.broadcasted_iota(jnp.int32, (G, d), 0)
        c = lax.broadcasted_iota(jnp.int32, (G, d), 1)
        same_head = (r // DH) == ((c % G) // DH)
        return jnp.where(same_head, tiled, 0.0).astype(jnp.bfloat16)

    def fold_group(bdt, w_s, out_ref, g):
        out_ref[g * G:(g + 1) * G, :] = lax.dot_general(
            bdt[:, g * G:(g + 1) * G], w_s[:, g * G:(g + 1) * G], _NT,
            preferred_element_type=jnp.float32).astype(out_ref.dtype)

    xc_off = [sum(X_CHUNKS[:i]) for i in range(len(X_CHUNKS))]

    def xc_copy(i):
        return pltpu.make_async_copy(x_hbm.at[pl.ds(xc_off[i], X_CHUNKS[i]), :],
                                     x_s.at[pl.ds(xc_off[i], X_CHUNKS[i]), :],
                                     sems.at[4 + len(WV_CHUNKS) + i])

    @pl.when(j == 0)
    def _():
        order = []
        for i in range(max(len(X_CHUNKS), len(WV_CHUNKS))):
            if i < len(X_CHUNKS):
                order.append(("x", i))
            if i < len(WV_CHUNKS):
                order.append(("w", i))

        def copy(item):
            return xc_copy(item[1]) if item[0] == "x" else wv_copy(item[1])

        for item in order[:AHEAD]:
            copy(item).start()
        kv_s[...] = jnp.zeros(kv_s.shape, kv_s.dtype)
        z_s[...] = jnp.zeros(z_s.shape, z_s.dtype)
        nx = 0
        nw = 0
        for k, item in enumerate(order):
            copy(item).wait()
            if k + AHEAD < len(order):
                copy(order[k + AHEAD]).start()
            if k + AHEAD == len(order):
                wphi_copy().start()
                wk_copy().start()
            if k == len(order) - 1:
                for blk in range(1, n_s):
                    x_copy(blk).start()
                wq_copy().start()
                wo_copy().start()
            if item[0] == "x":
                r0, r1 = xc_off[item[1]], xc_off[item[1]] + X_CHUNKS[item[1]]
                nx = r1
                if nw > 0:
                    v0_s[0:nw, r0:r1] = lax.dot_general(
                        wvt_s[0:nw, :], x_s[r0:r1, :], _NT,
                        preferred_element_type=jnp.float32).astype(jnp.bfloat16)
            else:
                lo, hi = wv_off[item[1]], wv_off[item[1]] + WV_CHUNKS[item[1]]
                nw = hi
                wt = wv_s[:, lo:hi].astype(jnp.float32).T.astype(jnp.bfloat16)
                wvt_s[lo:hi, :] = wt
                v0_s[lo:hi, 0:nx] = lax.dot_general(
                    wt, x_s[0:nx, :], _NT,
                    preferred_element_type=jnp.float32).astype(jnp.bfloat16)
        wphi_copy().wait()
        wk_copy().wait()
        bdt = bd_t()
        for g in range(ng):
            fold_group(bdt, wk_s, wkt_s, g)

    def phase1(first):
        x = load_x(j - 1)
        pk = lax.dot_general(wkt_s[...], x, _NT, preferred_element_type=jnp.float32)
        if first:
            vt = v0_s[...]
        else:
            vt = lax.dot_general(wvt_s[...], x, _NT,
                                 preferred_element_type=jnp.float32).astype(jnp.bfloat16)
        fp, fn = _dual_softmax_t(pk)
        zp = fp[:, 0:G]
        zn = fn[:, 0:G]
        for c in range(1, ts // G):
            zp = zp + fp[:, c * G:(c + 1) * G]
            zn = zn + fn[:, c * G:(c + 1) * G]
        z_s[0:d, :] += zp
        z_s[d:2 * d, :] += zn
        fpb = fp.astype(jnp.bfloat16)
        fnb = fn.astype(jnp.bfloat16)
        for p in range(npair):
            kv_s[p] += lax.dot_general(vt[2 * p * DH:(2 * p + 2) * DH], _pair_rhs(fpb, fnb, p),
                                       _NT, preferred_element_type=jnp.float32)

    @pl.when(j == 1)
    def _():
        phase1(True)

    @pl.when(jnp.logical_and(j >= 2, j <= n_s))
    def _():
        x_copy(j - 1).wait()
        phase1(False)

    @pl.when(j == n_s + 1)
    def _():
        wq_copy().wait()
        wo_copy().wait()
        bdt = bd_t()
        for g in range(ng):
            fold_group(bdt, wq_s, wqt_s, g)
        r = lax.broadcasted_iota(jnp.int32, (2 * DH, G), 0)
        c = lax.broadcasted_iota(jnp.int32, (2 * DH, G), 1)
        same_head = (r // DH) == (c // (2 * DH))
        for p in range(npair):
            lhs_s[p] = jnp.where(same_head, kv_s[p], 0.0).astype(jnp.bfloat16)
        zsum = jnp.sum(z_s[...], axis=1, keepdims=True)
        z_s[...] = jnp.broadcast_to(zsum, z_s.shape)

    @pl.when(j >= n_s + 1)
    def _():
        blk = j - 1 - n_s
        x = load_x(blk)
        pq = lax.dot_general(wqt_s[...], x, _NT, preferred_element_type=jnp.float32)
        fp, fn = _dual_softmax_t(pq)
        fpb = fp.astype(jnp.bfloat16)
        fnb = fn.astype(jnp.bfloat16)
        zp = z_s[0:d, :]
        zn = z_s[d:2 * d, :]
        dens = []
        for c in range(ts // G):
            t = fp[:, c * G:(c + 1) * G] * zp + fn[:, c * G:(c + 1) * G] * zn
            dens.append(jnp.sum(t.reshape(H, DH, G), axis=1, keepdims=True))
        rden = 1.0 / (jnp.concatenate(dens, axis=2) + 1e-6)
        outs = []
        for p in range(npair):
            r = lax.dot_general(lhs_s[p], _pair_rhs(fpb, fnb, p), _NN,
                                preferred_element_type=jnp.float32)
            num = r.reshape(2, DH, ts)
            outs.append((num * rden[2 * p:2 * p + 2]).reshape(2 * DH, ts))
        ot = jnp.concatenate(outs, axis=0)
        o = ot.T.astype(jnp.bfloat16)
        start = pl.multiple_of(blk * ts, ts)
        for c in range(noc):
            out_s[pl.ds(start, ts), c * OC:(c + 1) * OC] = lax.dot_general(
                o, wo_s[:, c * OC:(c + 1) * OC], _NN,
                preferred_element_type=jnp.float32).astype(out_s.dtype)
            out_copy(blk, c).start()

    @pl.when(j == 2 * n_s)
    def _():
        for blk in range(n_s):
            for c in range(noc):
                out_copy(blk, c).wait()


@jax.jit
def pallas_standalone__linear_kernel_hedgehog__prompt_kernel(x, wqkv, w_phi, wo):
    b, s, d = x.shape
    assert b == 1 and d == H * DH
    ts = sum(X_CHUNKS)
    assert s % ts == 0 and sum(WV_CHUNKS) == d
    n_s = s // ts
    x2 = x.reshape(s, d)
    wphi2 = w_phi.reshape(d, DH)
    kern = functools.partial(_kernel, n_s=n_s, ts=ts, d=d)
    out = pl.pallas_call(
        kern,
        grid=(2 * n_s + 1,),
        in_specs=[
            pl.BlockSpec(memory_space=pl.ANY),
            pl.BlockSpec(memory_space=pl.ANY),
            pl.BlockSpec(memory_space=pl.ANY),
            pl.BlockSpec(memory_space=pl.ANY),
        ],
        out_specs=pl.BlockSpec(memory_space=pl.ANY),
        out_shape=jax.ShapeDtypeStruct((s, d), x.dtype),
        scratch_shapes=[
            pltpu.VMEM((s, d), jnp.bfloat16),
            pltpu.VMEM((d, DH), jnp.bfloat16),
            pltpu.VMEM((d, d), jnp.bfloat16),
            pltpu.VMEM((d, d), jnp.bfloat16),
            pltpu.VMEM((d, d), jnp.bfloat16),
            pltpu.VMEM((d, d), jnp.bfloat16),
            pltpu.VMEM((d, d), jnp.bfloat16),
            pltpu.VMEM((d, d), jnp.bfloat16),
            pltpu.VMEM((d, d), jnp.bfloat16),
            pltpu.VMEM((d, ts), jnp.bfloat16),
            pltpu.VMEM((H // 2, 2 * DH, G), jnp.float32),
            pltpu.VMEM((2 * d, G), jnp.float32),
            pltpu.VMEM((H // 2, 2 * DH, G), jnp.bfloat16),
            pltpu.VMEM((s, d), jnp.bfloat16),
            pltpu.SemaphoreType.DMA((4 + len(WV_CHUNKS) + len(X_CHUNKS),)),
            pltpu.SemaphoreType.DMA((n_s,)),
            pltpu.SemaphoreType.DMA((n_s * (d // OC),)),
        ],
        compiler_params=pltpu.CompilerParams(
            dimension_semantics=("arbitrary",),
            vmem_limit_bytes=100 * 1024 * 1024,
        ),
    )(x2, wqkv, wphi2, wo)
    return out.reshape(b, s, d)
```
